```python
import os as _os
_os.environ.setdefault("JAX_PLATFORMS", "cpu")
import jax
import jax.numpy as jnp

def _softmax(x, axis=-1):
    return jax.nn.softmax(x, axis=axis)
def _gelu(x):
    return jax.nn.gelu(x, approximate=True)
def _silu(x):
    return jax.nn.silu(x)
def _sigmoid(x):
    return jax.nn.sigmoid(x)
def _layernorm(x, axis=-1, eps=1e-5):
    m = jnp.mean(x, axis=axis, keepdims=True)
    v = jnp.var(x, axis=axis, keepdims=True)
    return (x - m) / jnp.sqrt(v + eps)
def _scatter_add(tgt, idx, src, axis=0):
    return tgt.at[idx].add(src)
def _segment_sum(src, seg, n):
    return jax.ops.segment_sum(src, seg, n)
class _Rng:
    def __init__(self, key):
        self._k = key
    def _next(self):
        self._k, sub = jax.random.split(self._k)
        return sub
    def normal(self, shape):
        return jax.random.normal(self._next(), shape, dtype=jnp.bfloat16)
    def randint(self, lo, hi, shape):
        return jax.random.randint(self._next(), shape, lo, hi, dtype=jnp.int32)
    def uniform(self, shape, lo=0.0, hi=1.0):
        return jax.random.uniform(self._next(), shape, jnp.bfloat16, lo, hi)
    def permutation(self, n):
        return jax.random.permutation(self._next(), n)


kernel_name = 'parallel_sum__linear_kernel_hedgehog__dense_activation_gelu__prompt'

def setup_inputs():
    _rng = _Rng(jax.random.key(int.from_bytes(__import__("os").urandom(4), "little")))
    _w = (lambda a: (lambda t: t.astype(jnp.bfloat16) if jnp.issubdtype(t.dtype, jnp.floating) else t)(jnp.asarray(a)))
    def _A_setup():
        B, S, D, H = 1, 2048, 448, 16
        Dh = D // H
        return {
            "x": _w((lambda *s: _rng.normal(s) * 0.05)(B, S, D)),
            "wqkv": _w((lambda *s: _rng.normal(s) * 0.2)(D, 3 * D)),
            "w_phi": _w((lambda *s: _rng.normal(s) * 0.2)(H, Dh, Dh) * (Dh ** -0.5)),
            "wo": _w((lambda *s: _rng.normal(s) * 0.05)(D, D)),
        }
    _A_in = _A_setup()

    def _B_setup():
        B, S, D, F = 1, 2048, 448, 1792
        return {
            "x": _w((lambda *s: _rng.normal(s) * 0.05)(B, S, D)),
            "w1": _w((lambda *s: _rng.normal(s) * 0.2)(D, F) * (D ** -0.5)),
            "b1": _w((lambda *s: _rng.normal(s) * 0.2)(F) * 0.01),
            "w2": _w((lambda *s: _rng.normal(s) * 0.2)(F, D) * (F ** -0.5)),
            "b2": _w((lambda *s: _rng.normal(s) * 0.05)(D) * 0.01),
        }
    _B_in = _B_setup()

    return {
        "A_x": _A_in["x"],
        "A_wqkv": _A_in["wqkv"],
        "A_w_phi": _A_in["w_phi"],
        "A_wo": _A_in["wo"],
        "B_x": _B_in["x"],
        "B_w1": _B_in["w1"],
        "B_b1": _B_in["b1"],
        "B_w2": _B_in["w2"],
        "B_b2": _B_in["b2"],
    }

def reference(A_x, A_wqkv, A_w_phi, A_wo, B_x, B_w1, B_b1, B_w2, B_b2):
    def _A_ref(x, wqkv, w_phi, wo):
        B, S, D = x.shape
        H = 16; Dh = D // H
        qkv = (lambda x, *d: x.transpose(*d))((x @ wqkv).reshape(B, S, 3, H, Dh), 2, 0, 3, 1, 4)
        q, k, v = qkv[0], qkv[1], qkv[2]
        pq = jnp.einsum("bhsd,hdf->bhsf", q, w_phi)
        pk = jnp.einsum("bhsd,hdf->bhsf", k, w_phi)
        phi_q = jnp.concatenate([_softmax(pq, axis=-1), _softmax(-pq, axis=-1)], axis=-1)
        phi_k = jnp.concatenate([_softmax(pk, axis=-1), _softmax(-pk, axis=-1)], axis=-1)
        kv = jnp.einsum("bhsf,bhsd->bhfd", phi_k, v)
        z  = jnp.einsum("bhsf->bhf", phi_k)
        num = jnp.einsum("bhqf,bhfd->bhqd", phi_q, kv)
        den = jnp.einsum("bhqf,bhf->bhq", phi_q, z)[..., None] + 1e-6
        o = num / den
        return (lambda x, *d: x.transpose(*d))(o, 0, 2, 1, 3).reshape(B, S, D) @ wo

    def _B_ref(x, w1, b1, w2, b2):
        h = jnp.einsum("bsd,df->bsf", x, w1) + b1
        h = _gelu(h)
        return jnp.einsum("bsf,fd->bsd", h, w2) + b2

    x = A_x
    xn = _layernorm(x, axis=-1)
    return x + _A_ref(xn, A_wqkv, A_w_phi, A_wo) + _B_ref(xn, B_w1, B_b1, B_w2, B_b2)
```

```python
import functools
import math

import jax
import jax.numpy as jnp
import jax.experimental.pallas as pl
import jax.experimental.pallas.tpu as pltpu

S, D, H, DH, F = 2048, 448, 16, 28, 1792
KP = 512
NG = H // 2
GR = 2 * DH
QR = 4 * DH
NH = 2
EARLY = False
LOG2E = math.log2(math.e)
BF16 = jnp.bfloat16
F32 = jnp.float32
NT = (((1,), (1,)), ((), ()))


def _dot(a, b):
    return jnp.dot(a, b, preferred_element_type=F32)


def _dot_nt(a, b):
    return jax.lax.dot_general(a, b, NT, preferred_element_type=F32)


def _iota(shape, dim):
    return jax.lax.broadcasted_iota(jnp.int32, shape, dim)


def _recip(s):
    r = pl.reciprocal(s, approx=True)
    return r * (2.0 - s * r)


def _dual_softmax(p, sc):
    p3 = p.reshape(GR // 8, 8, sc)
    mx = jnp.max(p3, axis=0)
    mn = jnp.min(p3, axis=0)
    mx = jnp.maximum(mx, pltpu.roll(mx, 4, 0))
    mn = jnp.minimum(mn, pltpu.roll(mn, 4, 0))
    mx = jnp.maximum(mx, pltpu.roll(mx, 2, 0))
    mn = jnp.minimum(mn, pltpu.roll(mn, 2, 0))
    ep = jnp.exp2(p3 - mx[None])
    en = jnp.exp2(mn[None] - p3)
    sp = jnp.sum(ep, axis=0)
    sn = jnp.sum(en, axis=0)
    sp = sp + pltpu.roll(sp, 4, 0)
    sn = sn + pltpu.roll(sn, 4, 0)
    sp = sp + pltpu.roll(sp, 2, 0)
    sn = sn + pltpu.roll(sn, 2, 0)
    pp = (ep * _recip(sp)[None]).reshape(GR, sc)
    pn = (en * _recip(sn)[None]).reshape(GR, sc)
    return jnp.concatenate([pp, pn], axis=0).astype(BF16)


def _gelu(x):
    c = math.sqrt(2.0 / math.pi)
    inner = x * (c + (c * 0.044715) * (x * x))
    hx = 0.5 * x
    return hx + hx * jnp.tanh(inner)


def _kernel(xT_hbm, wqkv_hbm, wphi_hbm, wo_hbm, w1_hbm, b1_hbm, w2T_hbm, b2_hbm,
            outT_hbm,
            x_v, wqkv_v, wphi_v, a1_v, wc_v, woa_v, w2T_v, b1_v, b2_v,
            wA_v, wT_v, woT_v, xn_v, phiq_v, phik_v, vaug_v, kv_v, kvb_v, oT_v,
            out_v, xsem, wsem, csem, osem, *, sc, nc):
    nb = nc - 1
    cb = -(-F // (128 * nb)) * 128
    wc = nb * cb
    pad = KP - D

    def x_copy(c):
        return pltpu.make_async_copy(
            xT_hbm.at[:, pl.ds(c * sc, sc)], x_v.at[c], xsem.at[c])

    cp_wphi = pltpu.make_async_copy(wphi_hbm, wphi_v, wsem.at[0])
    cp_wk = pltpu.make_async_copy(
        wqkv_hbm.at[:, 384:896], wqkv_v.at[:, 384:896], wsem.at[1])
    cp_wv = pltpu.make_async_copy(
        wqkv_hbm.at[:, 896:1344], wqkv_v.at[:, 896:1344], wsem.at[2])
    cp_wq = pltpu.make_async_copy(
        wqkv_hbm.at[:, 0:384], wqkv_v.at[:, 0:384], wsem.at[3])
    cp_w2 = pltpu.make_async_copy(w2T_hbm, w2T_v, wsem.at[4])
    cp_b1 = pltpu.make_async_copy(b1_hbm, b1_v, wsem.at[5])
    cp_b2 = pltpu.make_async_copy(b2_hbm, b2_v, wsem.at[6])
    cp_wo = pltpu.make_async_copy(wo_hbm, woa_v.at[0:D, :], wsem.at[7])

    def w1_copy(b):
        lo, hi = b * cb, min((b + 1) * cb, F)
        return pltpu.make_async_copy(
            w1_hbm.at[:, lo:hi], wc_v.at[b, 0:D, 0:hi - lo], csem.at[b])

    def start_rest():
        for c in range(1, nc):
            x_copy(c).start()
            w1_copy(c - 1).start()
        cp_wo.start()
        cp_w2.start()

    cp_wphi.start()
    cp_wk.start()
    x_copy(0).start()
    if EARLY:
        start_rest()

    ones_row = jnp.where(_iota((pad, sc), 0) == 0, 1.0, 0.0).astype(BF16)
    for c in range(nc):
        xn_v[c, D:KP, :] = ones_row
        for g in range(NG):
            phiq_v[c, g, QR:128, :] = jnp.zeros((128 - QR, sc), BF16)
    oT_v[D:KP, :] = ones_row
    for g in range(NG):
        phik_v[g, QR:128, :] = jnp.zeros((128 - QR, sc), BF16)
    kv_v[...] = jnp.zeros(kv_v.shape, F32)
    wA_v[:, D:KP] = jnp.zeros((3 * D, pad), BF16)
    if wc > F:
        wc_v[nb - 1, 0:D, cb - (wc - F):cb] = jnp.zeros((D, wc - F), BF16)

    def layer_norm(c):
        for t in range(sc // 128):
            cs = slice(128 * t, 128 * t + 128)
            x = x_v[c, :, cs].astype(F32)
            mean = jnp.sum(x, axis=0, keepdims=True) * (1.0 / D)
            xc = x - mean
            var = jnp.sum(xc * xc, axis=0, keepdims=True) * (1.0 / D)
            xn_v[c, 0:D, cs] = (xc * jax.lax.rsqrt(var + 1e-5)).astype(BF16)

    cp_wphi.wait()
    r_i = _iota((D, D), 0)
    c_i = _iota((D, D), 1)
    perm = jnp.where(c_i == (r_i % DH) * H + r_i // DH, 1.0, 0.0).astype(BF16)
    a1_v[...] = _dot(perm, wphi_v[...]).astype(BF16)
    rsel = jnp.where((_iota((QR, DH), 0) % GR) // 2 == _iota((QR, DH), 1),
                     1.0, 0.0).astype(BF16)
    rr = _iota((QR, QR), 0)
    same_head = _iota((QR, QR), 1) // DH == 2 * (rr // GR) + rr % 2
    ls = [jnp.where(same_head, _dot_nt(rsel, a1_v[QR * q:QR * q + QR, :]),
                    0.0).astype(BF16) for q in range(4)]

    cp_wk.wait()
    cp_wq.start()
    cp_wv.start()
    cp_b1.start()
    cp_b2.start()
    for q in range(4):
        lo = D + QR * q
        wA_v[QR * q:QR * q + QR, 0:D] = (LOG2E * _dot_nt(
            ls[q], wqkv_v[:, lo:lo + QR])).astype(BF16)

    ones8 = jnp.ones((8, sc), F32)

    def kv_update():
        for g in range(NG):
            kv_v[g] += _dot_nt(vaug_v[g], phik_v[g])

    def proj_k(c):
        pk = _dot(wA_v[0:D, :], xn_v[c])
        for g in range(NG):
            phik_v[g, 0:QR, :] = _dual_softmax(pk[GR * g:GR * g + GR], sc)

    def proj_qv(c):
        pq = _dot(wA_v[D:2 * D, :], xn_v[c])
        for g in range(NG):
            phiq_v[c, g, 0:QR, :] = _dual_softmax(pq[GR * g:GR * g + GR], sc)
        vt = _dot(wA_v[2 * D:3 * D, :], xn_v[c])
        for g in range(NG):
            vaug_v[g] = jnp.concatenate(
                [vt[GR * g:GR * g + GR], ones8], axis=0).astype(BF16)

    x_copy(0).wait()
    layer_norm(0)
    proj_k(0)
    cp_wq.wait()
    cp_wv.wait()
    cp_b1.wait()
    cp_b2.wait()
    if not EARLY:
        start_rest()
    for q in range(4):
        lo = QR * q
        wA_v[D + QR * q:D + QR * q + QR, 0:D] = (LOG2E * _dot_nt(
            ls[q], wqkv_v[:, lo:lo + QR])).astype(BF16)
    wA_v[2 * D:3 * D, 0:D] = wqkv_v[:, 2 * D:3 * D].T
    b1 = b1_v[...].astype(F32).reshape(1, F)
    b2 = b2_v[...].astype(F32).reshape(1, D)
    if wc > F:
        b1 = jnp.concatenate([b1, jnp.zeros((1, wc - F), F32)], axis=1)
    bias_blk = jnp.where(_iota((pad, wc), 0) == 0,
                         jnp.broadcast_to(b1, (pad, wc)), 0.0).astype(BF16)
    for b in range(nb):
        wc_v[b, D:KP, :] = bias_blk[:, b * cb:(b + 1) * cb]
    woa_v[D:KP, :] = jnp.where(_iota((pad, D), 0) == 0,
                               jnp.broadcast_to(b2, (pad, D)), 0.0).astype(BF16)
    proj_qv(0)

    def loop_a(c, carry):
        x_copy(c).wait()
        for b in range(nb):
            @pl.when(c == b + 1)
            def _():
                w1_copy(b).wait()
        layer_norm(c)
        kv_update()
        proj_k(c)
        proj_qv(c)
        b = c - 1
        off = pl.multiple_of(b * cb, 128)
        wT_v[pl.ds(off, cb), :] = wc_v[b].T
        return carry

    jax.lax.fori_loop(1, nc, loop_a, 0)

    cp_wo.wait()
    cp_w2.wait()
    kv_update()
    woT_v[...] = woa_v[...].T

    r = _iota((64, 128), 0)
    jr = jnp.where(r < GR, r // DH, (r - GR) // 4)
    mask = jr == _iota((64, 128), 1) % 2
    for g in range(NG):
        kvb_v[g] = jnp.where(mask, kv_v[g], 0.0).astype(BF16)

    hs = sc // NH

    def out_copy(c, slot, k):
        return pltpu.make_async_copy(
            out_v.at[slot, :, k * hs:(k + 1) * hs],
            outT_hbm.at[:, pl.ds(c * sc + k * hs, hs)], osem.at[slot, k])

    sub = _iota((8, sc), 0) < 4

    def pass_b(c, carry):
        slot = c % 2

        @pl.when(c >= 2)
        def _():
            for k in range(NH):
                out_copy(c - 2, slot, k).wait()

        for q in range(4):
            parts = []
            for g in (2 * q, 2 * q + 1):
                oa = _dot(kvb_v[g], phiq_v[c, g])
                ra = 1.0 / (oa[GR:GR + 8] + 1e-6)
                ra_r = pltpu.roll(ra, 4, 0)
                r0 = jnp.where(sub, ra, ra_r)
                r1 = jnp.where(sub, ra_r, ra)
                scale = [r0, r0, r0, ra, r1, r1, r1]
                parts += [oa[8 * t:8 * t + 8] * scale[t] for t in range(7)]
            oT_v[QR * q:QR * q + QR, :] = jnp.concatenate(
                parts, axis=0).astype(BF16)
        h = _gelu(_dot(wT_v[0:F, :], xn_v[c])).astype(BF16)
        for k in range(NH):
            cs = slice(k * hs, (k + 1) * hs)
            acc = _dot(w2T_v[...], h[:, cs]) + _dot(woT_v[...], oT_v[:, cs])
            acc = acc + x_v[c, :, cs].astype(F32)
            out_v[slot, :, cs] = acc.astype(BF16)
            out_copy(c, slot, k).start()
        return carry

    jax.lax.fori_loop(0, nc, pass_b, 0)
    for k in range(NH):
        out_copy(nc - 2, nc % 2, k).wait()
        out_copy(nc - 1, (nc - 1) % 2, k).wait()


def _build(sc):
    nc = S // sc
    nb = nc - 1
    cb = -(-F // (128 * nb)) * 128
    any_spec = pl.BlockSpec(memory_space=pl.ANY)
    scratch = [
        pltpu.VMEM((nc, D, sc), BF16),
        pltpu.VMEM((D, 3 * D), BF16),
        pltpu.VMEM((D, DH), BF16),
        pltpu.VMEM((D, DH), BF16),
        pltpu.VMEM((nb, KP, cb), BF16),
        pltpu.VMEM((KP, D), BF16),
        pltpu.VMEM((D, F), BF16),
        pltpu.VMEM((F,), BF16),
        pltpu.VMEM((D,), BF16),
        pltpu.VMEM((3 * D, KP), BF16),
        pltpu.VMEM((nb * cb, KP), BF16),
        pltpu.VMEM((D, KP), BF16),
        pltpu.VMEM((nc, KP, sc), BF16),
        pltpu.VMEM((nc, NG, 128, sc), BF16),
        pltpu.VMEM((NG, 128, sc), BF16),
        pltpu.VMEM((NG, 64, sc), BF16),
        pltpu.VMEM((NG, 64, 128), F32),
        pltpu.VMEM((NG, 64, 128), BF16),
        pltpu.VMEM((KP, sc), BF16),
        pltpu.VMEM((2, D, sc), BF16),
        pltpu.SemaphoreType.DMA((nc,)),
        pltpu.SemaphoreType.DMA((8,)),
        pltpu.SemaphoreType.DMA((nb,)),
        pltpu.SemaphoreType.DMA((2, NH)),
    ]
    return pl.pallas_call(
        functools.partial(_kernel, sc=sc, nc=nc),
        out_shape=jax.ShapeDtypeStruct((D, S), BF16),
        in_specs=[any_spec] * 8,
        out_specs=any_spec,
        scratch_shapes=scratch,
        compiler_params=pltpu.CompilerParams(
            vmem_limit_bytes=100 * 1024 * 1024),
    )


@jax.jit
def pallas_parallel_sum__linear_kernel_hedgehog__dense_activation_gelu__prompt_kernel(
    A_x: jax.Array,
    A_wqkv: jax.Array,
    A_w_phi: jax.Array,
    A_wo: jax.Array,
    B_x: jax.Array,
    B_w1: jax.Array,
    B_b1: jax.Array,
    B_w2: jax.Array,
    B_b2: jax.Array,
):
    del B_x
    xT = A_x.reshape(S, D).T
    wphi = A_w_phi.transpose(1, 0, 2).reshape(DH * H, DH)
    outT = _build(512)(xT, A_wqkv, wphi, A_wo, B_w1, B_b1, B_w2.T, B_b2)
    return outT.T.reshape(1, S, D)
```

```python
import functools
import math

import jax
import jax.numpy as jnp
import jax.experimental.pallas as pl
import jax.experimental.pallas.tpu as pltpu

S, D, H, DH, F = 2048, 448, 16, 28, 1792
KP = 512
NG = H // 2
GR = 2 * DH
QR = 4 * DH
NH = 4
NR = 2
LOG2E = math.log2(math.e)
BF16 = jnp.bfloat16
F32 = jnp.float32
NT = (((1,), (1,)), ((), ()))


def _dot(a, b):
    return jnp.dot(a, b, preferred_element_type=F32)


def _dot_nt(a, b):
    return jax.lax.dot_general(a, b, NT, preferred_element_type=F32)


def _iota(shape, dim):
    return jax.lax.broadcasted_iota(jnp.int32, shape, dim)


def _recip(s):
    r = pl.reciprocal(s, approx=True)
    return r * (2.0 - s * r)


def _dual_softmax(p, w):
    p3 = p.reshape(GR // 8, 8, w)
    mx = jnp.max(p3, axis=0)
    mn = jnp.min(p3, axis=0)
    mx = jnp.maximum(mx, pltpu.roll(mx, 4, 0))
    mn = jnp.minimum(mn, pltpu.roll(mn, 4, 0))
    mx = jnp.maximum(mx, pltpu.roll(mx, 2, 0))
    mn = jnp.minimum(mn, pltpu.roll(mn, 2, 0))
    ep = jnp.exp2(p3 - mx[None])
    en = jnp.exp2(mn[None] - p3)
    sp = jnp.sum(ep, axis=0)
    sn = jnp.sum(en, axis=0)
    sp = sp + pltpu.roll(sp, 4, 0)
    sn = sn + pltpu.roll(sn, 4, 0)
    sp = sp + pltpu.roll(sp, 2, 0)
    sn = sn + pltpu.roll(sn, 2, 0)
    pp = (ep * _recip(sp)[None]).reshape(GR, w)
    pn = (en * _recip(sn)[None]).reshape(GR, w)
    return jnp.concatenate([pp, pn], axis=0).astype(BF16)


def _gelu(x):
    c = math.sqrt(2.0 / math.pi)
    inner = x * (c + (c * 0.044715) * (x * x))
    hx = 0.5 * x
    return hx + hx * jnp.tanh(inner)


def _kernel(xT_hbm, wqkv_hbm, wphi_hbm, wo_hbm, w1_hbm, b1_hbm, w2T_hbm, b2_hbm,
            outT_hbm,
            x_v, wqkv_v, wphi_v, a1_v, w1a_v, woa_v, w2T_v, b1_v, b2_v,
            wA_v, woT_v, xn_v, phiq_v, phik_v, vaug_v, kv_v, kvb_v, oT_v,
            out_v, xsem, wsem, osem, *, sc, nc):
    pad = KP - D

    def x_copy(c):
        return pltpu.make_async_copy(
            xT_hbm.at[:, pl.ds(c * sc, sc)], x_v.at[c], xsem.at[c])

    cp_wphi = pltpu.make_async_copy(wphi_hbm, wphi_v, wsem.at[0])
    cp_wk = pltpu.make_async_copy(
        wqkv_hbm.at[:, 384:896], wqkv_v.at[:, 384:896], wsem.at[1])
    cp_wv = pltpu.make_async_copy(
        wqkv_hbm.at[:, 896:1344], wqkv_v.at[:, 896:1344], wsem.at[2])
    cp_wq = pltpu.make_async_copy(
        wqkv_hbm.at[:, 0:384], wqkv_v.at[:, 0:384], wsem.at[2])
    cp_b1 = pltpu.make_async_copy(b1_hbm, b1_v, wsem.at[2])
    cp_b2 = pltpu.make_async_copy(b2_hbm, b2_v, wsem.at[2])
    cp_w1 = pltpu.make_async_copy(w1_hbm, w1a_v.at[0:D, :], wsem.at[3])
    cp_w2 = pltpu.make_async_copy(w2T_hbm, w2T_v, wsem.at[3])
    cp_wo = pltpu.make_async_copy(wo_hbm, woa_v.at[0:D, :], wsem.at[4])

    cp_wphi.start()
    cp_wk.start()
    x_copy(0).start()

    ones_row = jnp.where(_iota((pad, sc), 0) == 0, 1.0, 0.0).astype(BF16)
    for c in range(nc):
        xn_v[c, D:KP, :] = ones_row
        for g in range(NG):
            phiq_v[c, g, QR:128, :] = jnp.zeros((128 - QR, sc), BF16)
    oT_v[D:KP, :] = ones_row
    for g in range(NG):
        phik_v[g, QR:128, :] = jnp.zeros((128 - QR, sc), BF16)
    kv_v[...] = jnp.zeros(kv_v.shape, F32)
    wA_v[:, D:KP] = jnp.zeros((3 * D, pad), BF16)

    def layer_norm(c):
        tiles = []
        for t in range(sc // 128):
            cs = slice(128 * t, 128 * t + 128)
            x = x_v[c, :, cs].astype(F32)
            mean = jnp.sum(x, axis=0, keepdims=True) * (1.0 / D)
            xc = x - mean
            var = jnp.sum(xc * xc, axis=0, keepdims=True) * (1.0 / D)
            xn = (xc * jax.lax.rsqrt(var + 1e-5)).astype(BF16)
            xn_v[c, 0:D, cs] = xn
            tiles.append(xn)
        return jnp.concatenate(
            [jnp.concatenate(tiles, axis=1), ones_row], axis=0)

    cp_wphi.wait()
    r_i = _iota((D, D), 0)
    c_i = _iota((D, D), 1)
    perm = jnp.where(c_i == (r_i % DH) * H + r_i // DH, 1.0, 0.0).astype(BF16)
    a1_v[...] = _dot(perm, wphi_v[...]).astype(BF16)
    rsel = jnp.where((_iota((QR, DH), 0) % GR) // 2 == _iota((QR, DH), 1),
                     1.0, 0.0).astype(BF16)
    rr = _iota((QR, QR), 0)
    same_head = _iota((QR, QR), 1) // DH == 2 * (rr // GR) + rr % 2
    ls = [jnp.where(same_head, _dot_nt(rsel, a1_v[QR * q:QR * q + QR, :]),
                    0.0).astype(BF16) for q in range(4)]

    def fold_phi(row0, col0):
        for q in range(4):
            lo = col0 + QR * q
            wA_v[row0 + QR * q:row0 + QR * q + QR, 0:D] = (LOG2E * _dot_nt(
                ls[q], wqkv_v[:, lo:lo + QR])).astype(BF16)

    cp_wk.wait()
    cp_wq.start()
    cp_wv.start()
    cp_b1.start()
    cp_b2.start()
    fold_phi(0, D)

    ones8 = jnp.ones((8, sc), F32)

    def kv_update():
        for g in range(NG):
            kv_v[g] += _dot_nt(vaug_v[g], phik_v[g])

    def proj_k(xn):
        pk = _dot(wA_v[0:D, :], xn)
        for g in range(NG):
            phik_v[g, 0:QR, :] = _dual_softmax(pk[GR * g:GR * g + GR], sc)

    def proj_qv(c):
        pq = _dot(wA_v[D:2 * D, :], xn_v[c])
        for g in range(NG):
            phiq_v[c, g, 0:QR, :] = _dual_softmax(pq[GR * g:GR * g + GR], sc)
        vt = _dot(wA_v[2 * D:3 * D, :], xn_v[c])
        for g in range(NG):
            vaug_v[g] = jnp.concatenate(
                [vt[GR * g:GR * g + GR], ones8], axis=0).astype(BF16)

    x_copy(0).wait()
    xn0 = layer_norm(0)
    c1, c2 = sc - 256, sc - 128
    pk_a = _dot(wA_v[0:D, :], xn0[:, 0:c2])
    for g in range(NG):
        phik_v[g, 0:QR, 0:c1] = _dual_softmax(
            pk_a[GR * g:GR * g + GR, 0:c1], c1)
    cp_wq.wait()
    cp_wv.wait()
    cp_b1.wait()
    cp_b2.wait()
    for c in range(1, nc):
        x_copy(c).start()
    cp_wo.start()
    pk_b = _dot(wA_v[0:D, :], xn_v[0, :, c2:sc])
    for g in range(NG):
        phik_v[g, 0:QR, c1:c2] = _dual_softmax(
            pk_a[GR * g:GR * g + GR, c1:c2], 128)
        phik_v[g, 0:QR, c2:sc] = _dual_softmax(
            pk_b[GR * g:GR * g + GR], 128)
    fold_phi(D, 0)
    wA_v[2 * D:3 * D, 0:D] = wqkv_v[:, 2 * D:3 * D].T
    b1 = b1_v[...].astype(F32).reshape(1, F)
    b2 = b2_v[...].astype(F32).reshape(1, D)
    w1a_v[D:KP, :] = jnp.where(_iota((pad, F), 0) == 0,
                               jnp.broadcast_to(b1, (pad, F)), 0.0).astype(BF16)
    woa_v[D:KP, :] = jnp.where(_iota((pad, D), 0) == 0,
                               jnp.broadcast_to(b2, (pad, D)), 0.0).astype(BF16)
    proj_qv(0)

    for c in range(1, nc):
        if c == 1:
            for cc in range(1, nc):
                x_copy(cc).wait()
            cp_wo.wait()
            cp_w1.start()
            cp_w2.start()
        xn = layer_norm(c)
        kv_update()
        proj_k(xn)
        proj_qv(c)
        if c == 1:
            woT_v[...] = woa_v[...].T
    kv_update()

    r = _iota((64, 128), 0)
    jr = jnp.where(r < GR, r // DH, (r - GR) // 4)
    mask = jr == _iota((64, 128), 1) % 2
    for g in range(NG):
        kvb_v[g] = jnp.where(mask, kv_v[g], 0.0).astype(BF16)

    cp_w1.wait()
    cp_w2.wait()
    hs = sc // NH
    rs = D // NR

    def out_copy(c, k, r):
        return pltpu.make_async_copy(
            out_v.at[c, r * rs:(r + 1) * rs, k * hs:(k + 1) * hs],
            outT_hbm.at[r * rs:(r + 1) * rs, pl.ds(c * sc + k * hs, hs)],
            osem.at[0])

    sub = _iota((8, sc), 0) < 4

    def pass_b(c):
        for q in range(4):
            parts = []
            for g in (2 * q, 2 * q + 1):
                oa = _dot(kvb_v[g], phiq_v[c, g])
                ra = 1.0 / (oa[GR:GR + 8] + 1e-6)
                ra_r = pltpu.roll(ra, 4, 0)
                r0 = jnp.where(sub, ra, ra_r)
                r1 = jnp.where(sub, ra_r, ra)
                scale = [r0, r0, r0, ra, r1, r1, r1]
                parts += [oa[8 * t:8 * t + 8] * scale[t] for t in range(7)]
            oT_v[QR * q:QR * q + QR, :] = jnp.concatenate(
                parts, axis=0).astype(BF16)
        h = _gelu(_dot(xn_v[c].T, w1a_v[...])).astype(BF16)
        for k in range(NH):
            cs = slice(k * hs, (k + 1) * hs)
            acc = (_dot_nt(w2T_v[...], h[cs, :])
                   + _dot(woT_v[...], oT_v[:, cs]))
            for r in range(NR):
                rr = slice(r * rs, (r + 1) * rs)
                out_v[c, rr, cs] = (
                    acc[rr] + x_v[c, rr, cs].astype(F32)).astype(BF16)
                out_copy(c, k, r).start()

    def pass_b2(i, carry):
        pass_b(2 * i)
        pass_b(2 * i + 1)
        return carry

    jax.lax.fori_loop(0, nc // 2, pass_b2, 0)
    for c in range(nc):
        for k in range(NH):
            for r in range(NR):
                out_copy(c, k, r).wait()


def _build(sc):
    nc = S // sc
    any_spec = pl.BlockSpec(memory_space=pl.ANY)
    scratch = [
        pltpu.VMEM((nc, D, sc), BF16),
        pltpu.VMEM((D, 3 * D), BF16),
        pltpu.VMEM((D, DH), BF16),
        pltpu.VMEM((D, DH), BF16),
        pltpu.VMEM((KP, F), BF16),
        pltpu.VMEM((KP, D), BF16),
        pltpu.VMEM((D, F), BF16),
        pltpu.VMEM((F,), BF16),
        pltpu.VMEM((D,), BF16),
        pltpu.VMEM((3 * D, KP), BF16),
        pltpu.VMEM((D, KP), BF16),
        pltpu.VMEM((nc, KP, sc), BF16),
        pltpu.VMEM((nc, NG, 128, sc), BF16),
        pltpu.VMEM((NG, 128, sc), BF16),
        pltpu.VMEM((NG, 64, sc), BF16),
        pltpu.VMEM((NG, 64, 128), F32),
        pltpu.VMEM((NG, 64, 128), BF16),
        pltpu.VMEM((KP, sc), BF16),
        pltpu.VMEM((nc, D, sc), BF16),
        pltpu.SemaphoreType.DMA((nc,)),
        pltpu.SemaphoreType.DMA((5,)),
        pltpu.SemaphoreType.DMA((1,)),
    ]
    return pl.pallas_call(
        functools.partial(_kernel, sc=sc, nc=nc),
        out_shape=jax.ShapeDtypeStruct((D, S), BF16),
        in_specs=[any_spec] * 8,
        out_specs=any_spec,
        scratch_shapes=scratch,
        compiler_params=pltpu.CompilerParams(
            vmem_limit_bytes=100 * 1024 * 1024),
    )


@jax.jit
def pallas_parallel_sum__linear_kernel_hedgehog__dense_activation_gelu__prompt_kernel(
    A_x: jax.Array,
    A_wqkv: jax.Array,
    A_w_phi: jax.Array,
    A_wo: jax.Array,
    B_x: jax.Array,
    B_w1: jax.Array,
    B_b1: jax.Array,
    B_w2: jax.Array,
    B_b2: jax.Array,
):
    del B_x
    xT = A_x.reshape(S, D).T
    wphi = A_w_phi.transpose(1, 0, 2).reshape(DH * H, DH)
    outT = _build(512)(xT, A_wqkv, wphi, A_wo, B_w1, B_b1, B_w2.T, B_b2)
    return outT.T.reshape(1, S, D)
```

```python
import functools
import math

import jax
import jax.numpy as jnp
import jax.experimental.pallas as pl
import jax.experimental.pallas.tpu as pltpu

S, D, H, DH, F = 2048, 448, 16, 28, 1792
KP = 512
NG = H // 2
GR = 2 * DH
QR = 4 * DH
NH = 4
NR = 2
LOG2E = math.log2(math.e)
BF16 = jnp.bfloat16
F32 = jnp.float32
NT = (((1,), (1,)), ((), ()))


def _dot(a, b):
    return jnp.dot(a, b, preferred_element_type=F32)


def _dot_nt(a, b):
    return jax.lax.dot_general(a, b, NT, preferred_element_type=F32)


def _iota(shape, dim):
    return jax.lax.broadcasted_iota(jnp.int32, shape, dim)


def _colsum(x):
    w = x.shape[1]
    s = jnp.sum(x.reshape(7, 64, w), axis=0)
    s = jnp.sum(s.reshape(2, 32, w), axis=0)
    s = jnp.sum(s.reshape(2, 16, w), axis=0)
    s = jnp.sum(s.reshape(2, 8, w), axis=0)
    return jnp.sum(s, axis=0, keepdims=True)


def _recip(s):
    r = pl.reciprocal(s, approx=True)
    return r * (2.0 - s * r)


def _dual_softmax(p, w):
    p3 = p.reshape(GR // 8, 8, w)
    mx = jnp.max(p3, axis=0)
    mn = jnp.min(p3, axis=0)
    mx = jnp.maximum(mx, pltpu.roll(mx, 4, 0))
    mn = jnp.minimum(mn, pltpu.roll(mn, 4, 0))
    mx = jnp.maximum(mx, pltpu.roll(mx, 2, 0))
    mn = jnp.minimum(mn, pltpu.roll(mn, 2, 0))
    ep = jnp.exp2(p3 - mx[None])
    en = jnp.exp2(mn[None] - p3)
    sp = jnp.sum(ep, axis=0)
    sn = jnp.sum(en, axis=0)
    sp = sp + pltpu.roll(sp, 4, 0)
    sn = sn + pltpu.roll(sn, 4, 0)
    sp = sp + pltpu.roll(sp, 2, 0)
    sn = sn + pltpu.roll(sn, 2, 0)
    pp = (ep * _recip(sp)[None]).reshape(GR, w)
    pn = (en * _recip(sn)[None]).reshape(GR, w)
    return jnp.concatenate([pp, pn], axis=0).astype(BF16)


def _gelu(x):
    c = math.sqrt(2.0 / math.pi)
    inner = x * (c + (c * 0.044715) * (x * x))
    hx = 0.5 * x
    return hx + hx * jnp.tanh(inner)


def _kernel(xT_hbm, wqkv_hbm, wphi_hbm, wo_hbm, w1_hbm, b1_hbm, w2T_hbm, b2_hbm,
            outT_hbm,
            x_v, wqkv_v, wphi_v, a1_v, w1a_v, woa_v, w2T_v, b1_v, b2_v,
            wA_v, woT_v, xn_v, phiq_v, phik_v, vaug_v, kv_v, kvb_v, oT_v,
            out_v, xsem, wsem, osem, *, sc, nc):
    pad = KP - D

    def x_copy(c):
        return pltpu.make_async_copy(
            xT_hbm.at[:, pl.ds(c * sc, sc)], x_v.at[c], xsem.at[c])

    cp_wphi = pltpu.make_async_copy(wphi_hbm, wphi_v, wsem.at[0])
    cp_wk = pltpu.make_async_copy(
        wqkv_hbm.at[:, 384:896], wqkv_v.at[:, 384:896], wsem.at[1])
    cp_wv = pltpu.make_async_copy(
        wqkv_hbm.at[:, 896:1344], wqkv_v.at[:, 896:1344], wsem.at[2])
    cp_wq = pltpu.make_async_copy(
        wqkv_hbm.at[:, 0:384], wqkv_v.at[:, 0:384], wsem.at[2])
    cp_b1 = pltpu.make_async_copy(b1_hbm, b1_v, wsem.at[2])
    cp_b2 = pltpu.make_async_copy(b2_hbm, b2_v, wsem.at[2])
    cp_w1 = pltpu.make_async_copy(w1_hbm, w1a_v.at[0:D, :], wsem.at[3])
    cp_w2 = pltpu.make_async_copy(w2T_hbm, w2T_v, wsem.at[3])
    cp_wo = pltpu.make_async_copy(wo_hbm, woa_v.at[0:D, :], wsem.at[4])

    cp_wphi.start()
    cp_wk.start()
    x_copy(0).start()

    ones_row = jnp.where(_iota((pad, sc), 0) == 0, 1.0, 0.0).astype(BF16)
    for c in range(nc):
        xn_v[c, D:KP, :] = ones_row
        for g in range(NG):
            phiq_v[c, g, QR:128, :] = jnp.zeros((128 - QR, sc), BF16)
    oT_v[D:KP, :] = ones_row
    for g in range(NG):
        phik_v[g, QR:128, :] = jnp.zeros((128 - QR, sc), BF16)
    kv_v[...] = jnp.zeros(kv_v.shape, F32)
    wA_v[:, D:KP] = jnp.zeros((3 * D, pad), BF16)

    def layer_norm(c, nfast=0):
        tiles = []
        for t in range(sc // 128):
            cs = slice(128 * t, 128 * t + 128)
            x = x_v[c, :, cs].astype(F32)
            if t < nfast:
                csum = _colsum
            else:
                csum = functools.partial(jnp.sum, axis=0, keepdims=True)
            mean = csum(x) * (1.0 / D)
            xc = x - mean
            var = csum(xc * xc) * (1.0 / D)
            xn = (xc * jax.lax.rsqrt(var + 1e-5)).astype(BF16)
            xn_v[c, 0:D, cs] = xn
            tiles.append(xn)
        return jnp.concatenate(
            [jnp.concatenate(tiles, axis=1), ones_row], axis=0)

    cp_wphi.wait()
    r_i = _iota((D, D), 0)
    c_i = _iota((D, D), 1)
    perm = jnp.where(c_i == (r_i % DH) * H + r_i // DH, 1.0, 0.0).astype(BF16)
    a1_v[...] = _dot(perm, wphi_v[...]).astype(BF16)
    rsel = jnp.where((_iota((QR, DH), 0) % GR) // 2 == _iota((QR, DH), 1),
                     1.0, 0.0).astype(BF16)
    rr = _iota((QR, QR), 0)
    same_head = _iota((QR, QR), 1) // DH == 2 * (rr // GR) + rr % 2
    ls = [jnp.where(same_head, _dot_nt(rsel, a1_v[QR * q:QR * q + QR, :]),
                    0.0).astype(BF16) for q in range(4)]

    def fold_phi(row0, col0):
        for q in range(4):
            lo = col0 + QR * q
            wA_v[row0 + QR * q:row0 + QR * q + QR, 0:D] = (LOG2E * _dot_nt(
                ls[q], wqkv_v[:, lo:lo + QR])).astype(BF16)

    cp_wk.wait()
    cp_wq.start()
    cp_wv.start()
    cp_b1.start()
    cp_b2.start()
    fold_phi(0, D)

    ones8 = jnp.ones((8, sc), F32)

    def kv_update():
        for g in range(NG):
            kv_v[g] += _dot_nt(vaug_v[g], phik_v[g])

    def proj_k(xn):
        pk = _dot(wA_v[0:D, :], xn)
        for g in range(NG):
            phik_v[g, 0:QR, :] = _dual_softmax(pk[GR * g:GR * g + GR], sc)

    def proj_q(c):
        pq = _dot(wA_v[D:2 * D, :], xn_v[c])
        for g in range(NG):
            phiq_v[c, g, 0:QR, :] = _dual_softmax(pq[GR * g:GR * g + GR], sc)

    def proj_v(xn):
        vt = _dot(wA_v[2 * D:3 * D, :], xn)
        for g in range(NG):
            vaug_v[g] = jnp.concatenate(
                [vt[GR * g:GR * g + GR], ones8], axis=0).astype(BF16)

    x_copy(0).wait()
    xn0 = layer_norm(0, 1)
    c1, c2 = sc - 256, sc - 128
    pk_a = _dot(wA_v[0:D, :], xn0[:, 0:c2])
    for g in range(NG):
        phik_v[g, 0:QR, 0:c1] = _dual_softmax(
            pk_a[GR * g:GR * g + GR, 0:c1], c1)
    cp_wq.wait()
    cp_wv.wait()
    cp_b1.wait()
    cp_b2.wait()
    for c in range(1, nc):
        x_copy(c).start()
    cp_wo.start()
    pk_b = _dot(wA_v[0:D, :], xn_v[0, :, c2:sc])
    for g in range(NG):
        phik_v[g, 0:QR, c1:c2] = _dual_softmax(
            pk_a[GR * g:GR * g + GR, c1:c2], 128)
        phik_v[g, 0:QR, c2:sc] = _dual_softmax(
            pk_b[GR * g:GR * g + GR], 128)
    fold_phi(D, 0)
    wA_v[2 * D:3 * D, 0:D] = wqkv_v[:, 2 * D:3 * D].T
    b1 = b1_v[...].astype(F32).reshape(1, F)
    b2 = b2_v[...].astype(F32).reshape(1, D)
    w1a_v[D:KP, :] = jnp.where(_iota((pad, F), 0) == 0,
                               jnp.broadcast_to(b1, (pad, F)), 0.0).astype(BF16)
    woa_v[D:KP, :] = jnp.where(_iota((pad, D), 0) == 0,
                               jnp.broadcast_to(b2, (pad, D)), 0.0).astype(BF16)
    proj_q(0)
    proj_v(xn_v[0])

    for c in range(1, nc):
        if c == 1:
            for cc in range(1, nc):
                x_copy(cc).wait()
            cp_wo.wait()
            cp_w1.start()
            cp_w2.start()
        xn = layer_norm(c)
        kv_update()
        proj_v(xn)
        proj_k(xn_v[c])
        proj_q(c)
        if c == 1:
            woT_v[...] = woa_v[...].T
    kv_update()

    r = _iota((64, 128), 0)
    jr = jnp.where(r < GR, r // DH, (r - GR) // 4)
    mask = jr == _iota((64, 128), 1) % 2
    for g in range(NG):
        kvb_v[g] = jnp.where(mask, kv_v[g], 0.0).astype(BF16)

    cp_w1.wait()
    cp_w2.wait()
    hs = sc // NH
    rs = D // NR

    def out_copy(c, k, r):
        return pltpu.make_async_copy(
            out_v.at[c, r * rs:(r + 1) * rs, k * hs:(k + 1) * hs],
            outT_hbm.at[r * rs:(r + 1) * rs, pl.ds(c * sc + k * hs, hs)],
            osem.at[0])

    sub = _iota((8, sc), 0) < 4

    def pass_b(c):
        for q in range(4):
            parts = []
            for g in (2 * q, 2 * q + 1):
                oa = _dot(kvb_v[g], phiq_v[c, g])
                ra = 1.0 / (oa[GR:GR + 8] + 1e-6)
                ra_r = pltpu.roll(ra, 4, 0)
                r0 = jnp.where(sub, ra, ra_r)
                r1 = jnp.where(sub, ra_r, ra)
                scale = [r0, r0, r0, ra, r1, r1, r1]
                parts += [oa[8 * t:8 * t + 8] * scale[t] for t in range(7)]
            oT_v[QR * q:QR * q + QR, :] = jnp.concatenate(
                parts, axis=0).astype(BF16)
        h = _gelu(_dot(xn_v[c].T, w1a_v[...])).astype(BF16)
        for k in range(NH):
            cs = slice(k * hs, (k + 1) * hs)
            acc = (_dot_nt(w2T_v[...], h[cs, :])
                   + _dot(woT_v[...], oT_v[:, cs]))
            for r in range(NR):
                rr = slice(r * rs, (r + 1) * rs)
                out_v[c, rr, cs] = (
                    acc[rr] + x_v[c, rr, cs].astype(F32)).astype(BF16)
                out_copy(c, k, r).start()

    def pass_b2(i, carry):
        pass_b(2 * i)
        pass_b(2 * i + 1)
        return carry

    jax.lax.fori_loop(0, nc // 2, pass_b2, 0)
    for c in range(nc):
        for k in range(NH):
            for r in range(NR):
                out_copy(c, k, r).wait()


def _build(sc):
    nc = S // sc
    any_spec = pl.BlockSpec(memory_space=pl.ANY)
    scratch = [
        pltpu.VMEM((nc, D, sc), BF16),
        pltpu.VMEM((D, 3 * D), BF16),
        pltpu.VMEM((D, DH), BF16),
        pltpu.VMEM((D, DH), BF16),
        pltpu.VMEM((KP, F), BF16),
        pltpu.VMEM((KP, D), BF16),
        pltpu.VMEM((D, F), BF16),
        pltpu.VMEM((F,), BF16),
        pltpu.VMEM((D,), BF16),
        pltpu.VMEM((3 * D, KP), BF16),
        pltpu.VMEM((D, KP), BF16),
        pltpu.VMEM((nc, KP, sc), BF16),
        pltpu.VMEM((nc, NG, 128, sc), BF16),
        pltpu.VMEM((NG, 128, sc), BF16),
        pltpu.VMEM((NG, 64, sc), BF16),
        pltpu.VMEM((NG, 64, 128), F32),
        pltpu.VMEM((NG, 64, 128), BF16),
        pltpu.VMEM((KP, sc), BF16),
        pltpu.VMEM((nc, D, sc), BF16),
        pltpu.SemaphoreType.DMA((nc,)),
        pltpu.SemaphoreType.DMA((5,)),
        pltpu.SemaphoreType.DMA((1,)),
    ]
    return pl.pallas_call(
        functools.partial(_kernel, sc=sc, nc=nc),
        out_shape=jax.ShapeDtypeStruct((D, S), BF16),
        in_specs=[any_spec] * 8,
        out_specs=any_spec,
        scratch_shapes=scratch,
        compiler_params=pltpu.CompilerParams(
            vmem_limit_bytes=100 * 1024 * 1024),
    )


@jax.jit
def pallas_parallel_sum__linear_kernel_hedgehog__dense_activation_gelu__prompt_kernel(
    A_x: jax.Array,
    A_wqkv: jax.Array,
    A_w_phi: jax.Array,
    A_wo: jax.Array,
    B_x: jax.Array,
    B_w1: jax.Array,
    B_b1: jax.Array,
    B_w2: jax.Array,
    B_b2: jax.Array,
):
    del B_x
    xT = A_x.reshape(S, D).T
    wphi = A_w_phi.transpose(1, 0, 2).reshape(DH * H, DH)
    outT = _build(512)(xT, A_wqkv, wphi, A_wo, B_w1, B_b1, B_w2.T, B_b2)
    return outT.T.reshape(1, S, D)
```
